```python
import jax
import jax.numpy as jnp

def _softmax(x, axis=-1):
    return jax.nn.softmax(x, axis=axis)
def _gelu(x):
    return jax.nn.gelu(x, approximate=True)
def _silu(x):
    return jax.nn.silu(x)
def _sigmoid(x):
    return jax.nn.sigmoid(x)
def _layernorm(x, axis=-1, eps=1e-5):
    m = jnp.mean(x, axis=axis, keepdims=True)
    v = jnp.var(x, axis=axis, keepdims=True)
    return (x - m) / jnp.sqrt(v + eps)
def _scatter_add(tgt, idx, src, axis=0):
    return tgt.at[idx].add(src)
def _segment_sum(src, seg, n):
    return jax.ops.segment_sum(src, seg, n)
class _Rng:
    def __init__(self, key):
        self._k = key
    def _next(self):
        self._k, sub = jax.random.split(self._k)
        return sub
    def normal(self, shape):
        return jax.random.normal(self._next(), shape, dtype=jnp.bfloat16)
    def randint(self, lo, hi, shape):
        return jax.random.randint(self._next(), shape, lo, hi, dtype=jnp.int32)
    def uniform(self, shape, lo=0.0, hi=1.0):
        return jax.random.uniform(self._next(), shape, jnp.bfloat16, lo, hi)
    def permutation(self, n):
        return jax.random.permutation(self._next(), n)


kernel_name = 'concat_heads__ssm_conv_h3__linear_attn_block__prompt'

def setup_inputs():
    _rng = _Rng(jax.random.key(int.from_bytes(__import__("os").urandom(4), "little")))
    _w = (lambda a: (lambda t: t.astype(jnp.bfloat16) if jnp.issubdtype(t.dtype, jnp.floating) else t)(jnp.asarray(a)))
    def _A_setup():
        B, S, D = 1, 2048, 1024
        ks = 4
        return {
            "q": _w((lambda *s: _rng.normal(s) * 0.05)(B, S, D)),
            "k": _w((lambda *s: _rng.normal(s) * 0.05)(B, S, D)),
            "v": _w((lambda *s: _rng.normal(s) * 0.05)(B, S, D)),
            "shift_k": _w((lambda *s: _rng.normal(s) * 0.05)(D, ks) * 0.5),
            "ssm_k": _w((lambda *s: _rng.normal(s) * 0.05)(D, S) * (1.0 / S ** 0.5)),
            "ssm_D": _w((lambda *s: _rng.normal(s) * 0.05)(D)),
        }
    _A_in = _A_setup()

    def _B_setup():
        B, S, D = 1, 2048, 1024
        return {
            "x": _w((lambda *s: _rng.normal(s) * 0.05)(B, S, D)),
            "wqkv": _w((lambda *s: _rng.normal(s) * 0.05)(D, 3 * D)),
            "wo": _w((lambda *s: _rng.normal(s) * 0.05)(D, D)),
        }
    _B_in = _B_setup()

    return {
        "A_q": _A_in["q"],
        "A_k": _A_in["k"],
        "A_v": _A_in["v"],
        "A_shift_k": _A_in["shift_k"],
        "A_ssm_k": _A_in["ssm_k"],
        "A_ssm_D": _A_in["ssm_D"],
        "B_x": _B_in["x"],
        "B_wqkv": _B_in["wqkv"],
        "B_wo": _B_in["wo"],
    }

def reference(A_q, A_k, A_v, A_shift_k, A_ssm_k, A_ssm_D, B_x, B_wqkv, B_wo):
    def _A_ref(q, k, v, shift_k, ssm_k, ssm_D):
        B, S, D = q.shape
        ks = shift_k.shape[-1]
        k_pad = jnp.pad(k, ((0, 0), (ks - 1, 0), (0, 0)))
        k_shift = jnp.zeros_like(k)
        for t in range(ks):
            k_shift = k_shift + k_pad[:, t:t + S, :] * shift_k[:, ks - 1 - t][None, None, :]
        kv = k_shift * v
        L = 2 * S
        kv_pad = jnp.pad(kv, ((0, 0), (0, S), (0, 0)))
        kf_pad = jnp.pad(ssm_k, ((0, 0), (0, S)))
        kv_f = (lambda x, axes=(-2,-1): jnp.fft.rfft2(x.astype(jnp.float32), axes=axes))(kv_pad[:, None, :, :], axes=(1, 2))
        kf_f = (lambda x, axes=(-2,-1): jnp.fft.rfft2(x.astype(jnp.float32), axes=axes))(kf_pad[:, None, :], axes=(1, 2))
        kf_f = (lambda x, *d: x.transpose(*d))(kf_f, 1, 2, 0)
        y_f = kv_f * kf_f[None, :, :, :]
        y = (lambda x, s, axes=(-2,-1): jnp.fft.irfft2(x, s=s, axes=axes).astype(jnp.bfloat16))(y_f, (1, L), axes=(1, 2))[:, 0, :S, :]
        y = y + kv * ssm_D[None, None, :]
        return q * y

    def _B_ref(x, wqkv, wo):
        B, S, D = x.shape
        H = 32; Dh = D // H
        qkv = (lambda x, *d: x.transpose(*d))((x @ wqkv).reshape(B, S, 3, H, Dh), 2, 0, 3, 1, 4)
        q, k, v = qkv[0], qkv[1], qkv[2]
        phi = lambda t: jnp.where(t > 0, t + 1, jnp.exp(t)) + 1e-6
        pq, pk = phi(q), phi(k)
        kv = jnp.einsum("bhsd,bhse->bhde", pk, v)
        z = jnp.einsum("bhsd->bhd", pk)
        num = jnp.einsum("bhqd,bhde->bhqe", pq, kv)
        den = jnp.einsum("bhqd,bhd->bhq", pq, z)[..., None] + 1e-6
        o = num / den
        return (lambda x, *d: x.transpose(*d))(o, 0, 2, 1, 3).reshape(B, S, D) @ wo

    a = _A_ref(A_q, A_k, A_v, A_shift_k, A_ssm_k, A_ssm_D)
    b = _B_ref(B_x, B_wqkv, B_wo)
    return jnp.concatenate([a, b], axis=-1)
```

```python
import functools
import jax
import jax.numpy as jnp
import numpy as np
import ml_dtypes
from jax import lax
import jax.experimental.pallas as pl
import jax.experimental.pallas.tpu as pltpu

S, D = 2048, 1024
NT = D // 128
CH = 512
NC = S // CH
F32, BF16, U32, I32 = jnp.float32, jnp.bfloat16, jnp.uint32, jnp.int32


def _consts():
    k1 = np.arange(128)
    n1 = np.arange(128)
    W1 = np.zeros((16, 256, 128), np.float64)
    WI = np.zeros((16, 128, 256), np.float64)
    row_re = 16 * (k1 // 8) + (k1 % 8)
    row_im = row_re + 8
    for n2 in range(16):
        ang = 2 * np.pi * (k1[:, None] + 0.25) * (16 * n1[None, :] + n2) / 2048.0
        W1[n2, row_re] = np.cos(ang)
        W1[n2, row_im] = -np.sin(ang)
        WI[n2][:, row_re] = np.cos(ang).T / 2048.0
        WI[n2][:, row_im] = -np.sin(ang).T / 2048.0
    return W1.astype(ml_dtypes.bfloat16), WI.astype(ml_dtypes.bfloat16)


def _r4(x0, x1, x2, x3, inv):
    s02 = (x0[0] + x2[0], x0[1] + x2[1])
    d02 = (x0[0] - x2[0], x0[1] - x2[1])
    s13 = (x1[0] + x3[0], x1[1] + x3[1])
    d13 = (x1[0] - x3[0], x1[1] - x3[1])
    y0 = (s02[0] + s13[0], s02[1] + s13[1])
    y2 = (s02[0] - s13[0], s02[1] - s13[1])
    ya = (d02[0] + d13[1], d02[1] - d13[0])
    yb = (d02[0] - d13[1], d02[1] + d13[0])
    return (y0, yb, y2, ya) if inv else (y0, ya, y2, yb)


def _tw(x, e, inv):
    e = e % 16
    if inv:
        e = (16 - e) % 16
    r, i = x
    if e == 0:
        return x
    if e == 4:
        return (i, -r)
    if e == 12:
        return (-i, r)
    c = float(np.cos(2 * np.pi * e / 16))
    s = float(np.sin(2 * np.pi * e / 16))
    if e % 4 == 2:
        if np.sign(c) == np.sign(s):
            return ((r + i) * c, (i - r) * c)
        return ((r - i) * c, (i + r) * c)
    return (r * c + i * s, i * c - r * s)


def _fft16(x, inv):
    T = [None] * 4
    for b in range(4):
        y = _r4(x[b], x[4 + b], x[8 + b], x[12 + b], inv)
        T[b] = [_tw(y[ka], b * ka, inv) for ka in range(4)]
    out = [None] * 16
    for ka in range(4):
        y = _r4(T[0][ka], T[1][ka], T[2][ka], T[3][ka], inv)
        for kb in range(4):
            out[ka + 4 * kb] = y[kb]
    return out


def _lo(u):
    return pltpu.unpack_elementwise(u, index=0, packed_dtype=BF16, unpacked_dtype=F32)


def _hi(u):
    return pltpu.unpack_elementwise(u, index=1, packed_dtype=BF16, unpacked_dtype=F32)


def _phi(t):
    return jnp.where(t > 0, t + 1.0, jnp.exp(t)) + 1e-6


def _kernel(q_h, k_h, v_h, sk_h, h_h, sd_h, x_h, w_h, wo_h, w1_h, wi_h,
            o_h,
            qb, kb, vb, hb, skb, sdb, xb, wb, wob, w1b, wib,
            ht, kvb, xa, hf, pb, oa, kvs, zs, kvw, zb, pqb, ob,
            sem_in, sem_a, sem_o):
    def cp(src, dst, sem):
        return pltpu.make_async_copy(src, dst, sem)

    def a_copies(t):
        cs = pl.ds(pl.multiple_of(t * 128, 128), 128)
        return [
            cp(k_h.at[:, cs], kb.at[t, pl.ds(16, S)], sem_a.at[t, 0]),
            cp(v_h.at[:, cs], vb.at[t], sem_a.at[t, 1]),
            cp(h_h.at[cs, :], hb.at[t], sem_a.at[t, 2]),
            cp(q_h.at[:, cs], qb.at[t], sem_a.at[t, 3]),
        ]
    c_small = [cp(sk_h, skb, sem_in.at[0]), cp(sd_h, sdb, sem_in.at[1]),
               cp(w1_h, w1b, sem_in.at[2]), cp(wi_h, wib, sem_in.at[3])]
    c_x = [cp(x_h.at[:, pl.ds(t * 128, 128)], xb.at[t], sem_in.at[4 + t]) for t in range(NT)]
    c_w = [cp(w_h.at[:, pl.ds(n * 128, 128)], wb.at[n], sem_in.at[12 + n]) for n in range(3 * NT)]
    c_wo = [cp(wo_h.at[:, pl.ds(n * 128, 128)], wob.at[n], sem_in.at[36 + n]) for n in range(NT)]
    for c in c_small:
        c.start()
    for c in a_copies(0):
        c.start()
    for c in c_x + c_w:
        c.start()
    for t in range(1, NT):
        for c in a_copies(t):
            c.start()
    for c in c_wo:
        c.start()
    for t in range(NT):
        kb[t, 0:16, :] = jnp.zeros((16, 128), BF16)
    for c in c_small:
        c.wait()

    kbu = kb.bitcast(U32)
    vbu = vb.bitcast(U32)
    qbu = qb.bitcast(U32)
    htu = ht.bitcast(U32)
    oau = oa.bitcast(U32)

    def a_tile(t, carry):
        for c in a_copies(t):
            c.wait()
        w = [skb[t, j:j + 1, :] for j in range(4)]
        for j in range(8):
            base = 8 * 16 * j + 8
            kk = {}
            for m in range(-2, 8):
                u = kbu[t, pl.ds(base + m, 16, stride=8), :]
                kk[2 * m] = _lo(u)
                kk[2 * m + 1] = _hi(u)
            for m in range(8):
                u = vbu[t, pl.ds(base - 8 + m, 16, stride=8), :]
                for n2, vv in ((2 * m, _lo(u)), (2 * m + 1, _hi(u))):
                    ks = kk[n2] * w[0] + kk[n2 - 1] * w[1] + kk[n2 - 2] * w[2] + kk[n2 - 3] * w[3]
                    kvb[n2, 16 * j:16 * j + 16, 0:128] = (ks * vv).astype(BF16)
        ht[...] = hb[t].T
        for m in range(8):
            u = htu[pl.ds(m, 128, stride=8), :]
            kvb[2 * m, :, 128:256] = _lo(u).astype(BF16)
            kvb[2 * m + 1, :, 128:256] = _hi(u).astype(BF16)
        for n2 in range(16):
            xa[n2] = jnp.dot(w1b[n2], kvb[n2], preferred_element_type=F32)
        for g in range(16):
            r0, r1, r2 = 16 * g, 16 * g + 8, 16 * g + 16
            H = _fft16([(xa[n, r0:r1, 128:256], xa[n, r1:r2, 128:256]) for n in range(16)], False)
            X = _fft16([(xa[n, r0:r1, 0:128], xa[n, r1:r2, 0:128]) for n in range(16)], False)
            P = [(X[n][0] * H[n][0] - X[n][1] * H[n][1], X[n][0] * H[n][1] + X[n][1] * H[n][0])
                 for n in range(16)]
            Y = _fft16(P, True)
            for n in range(16):
                pb[n, r0:r2, :] = jnp.concatenate(Y[n], axis=0).astype(BF16)
        dd = sdb[t]
        for m in range(8):
            u = qbu[t, pl.ds(m, 128, stride=8), :]
            res = []
            for n2, qq in ((2 * m, _lo(u)), (2 * m + 1, _hi(u))):
                y = jnp.dot(wib[n2], pb[n2], preferred_element_type=F32)
                y = y + kvb[n2, :, 0:128].astype(F32) * dd
                res.append(y * qq)
            oau[t, pl.ds(m, 128, stride=8), :] = pltpu.pack_elementwise(res, packed_dtype=BF16)
        cs = pl.ds(pl.multiple_of(t * 128, 128), 128)
        cp(oa.at[t], o_h.at[:, cs], sem_o.at[0, t]).start()
        return carry

    lax.fori_loop(0, NT, a_tile, 0)

    for c in c_x + c_w:
        c.wait()
    kvs[...] = jnp.zeros(kvs.shape, F32)
    zs[...] = jnp.zeros(zs.shape, F32)

    def proj(rows, n):
        acc = None
        for k in range(NT):
            p = jnp.dot(xb[k, rows, :], wb[n, k * 128:(k + 1) * 128, :], preferred_element_type=F32)
            acc = p if acc is None else acc + p
        return acc

    def b1(c, carry):
        rows = pl.ds(pl.multiple_of(c * CH, CH), CH)
        for n in range(NT):
            pk = _phi(proj(rows, NT + n))
            zs[n] += jnp.sum(pk.reshape(CH // 8, 8, 128), axis=0)
            vv = proj(rows, 2 * NT + n).astype(BF16)
            kvs[n] += lax.dot_general(pk.astype(BF16), vv, (((0,), (0,)), ((), ())),
                                      preferred_element_type=F32)
        return carry

    lax.fori_loop(0, NC, b1, 0)

    for c in c_wo:
        c.wait()
    ri = lax.broadcasted_iota(I32, (128, 128), 0)
    ci = lax.broadcasted_iota(I32, (128, 128), 1)
    mask = (ri // 32) == (ci // 32)
    for g in range(NT):
        kvm = jnp.where(mask, kvs[g], 0.0).astype(BF16)
        for n in range(NT):
            kvw[n, g * 128:(g + 1) * 128, :] = jnp.dot(
                kvm, wob[n, g * 128:(g + 1) * 128, :], preferred_element_type=F32).astype(BF16)
        z = jnp.sum(zs[g], axis=0, keepdims=True)
        zt = jnp.broadcast_to(z, (128, 128)).T
        zb[g] = jnp.where(mask, zt, 0.0).astype(BF16)

    def b3(c, carry):
        rows = pl.ds(pl.multiple_of(c * CH, CH), CH)
        for g in range(NT):
            pq = _phi(proj(rows, g)).astype(BF16)
            den = jnp.dot(pq, zb[g], preferred_element_type=F32) + 1e-6
            pqb[g] = (pq.astype(F32) / den).astype(BF16)
        for n in range(NT):
            acc = None
            for g in range(NT):
                p = jnp.dot(pqb[g], kvw[n, g * 128:(g + 1) * 128, :], preferred_element_type=F32)
                acc = p if acc is None else acc + p
            ob[n, rows, :] = acc.astype(BF16)
            cp(ob.at[n, rows], o_h.at[rows, pl.ds(D + n * 128, 128)], sem_o.at[1 + c, n]).start()
        return carry

    lax.fori_loop(0, NC, b3, 0)

    for t in range(NT):
        cp(oa.at[t], o_h.at[:, pl.ds(t * 128, 128)], sem_o.at[0, t]).wait()
        for c in range(NC):
            rows = pl.ds(c * CH, CH)
            cp(ob.at[t, rows], o_h.at[rows, pl.ds(D + t * 128, 128)], sem_o.at[1 + c, t]).wait()


@jax.jit
def pallas_concat_heads__ssm_conv_h3__linear_attn_block__prompt_kernel(
        A_q, A_k, A_v, A_shift_k, A_ssm_k, A_ssm_D, B_x, B_wqkv, B_wo):
    W1, WI = _consts()
    sk = A_shift_k.T.astype(F32).reshape(4, NT, 128).transpose(1, 0, 2)
    sd = A_ssm_D.astype(F32).reshape(NT, 1, 128)
    any_spec = pl.BlockSpec(memory_space=pl.ANY)
    scratch = [
        pltpu.VMEM((NT, S, 128), BF16),
        pltpu.VMEM((NT, S + 16, 128), BF16),
        pltpu.VMEM((NT, S, 128), BF16),
        pltpu.VMEM((NT, 128, S), BF16),
        pltpu.VMEM((NT, 4, 128), F32),
        pltpu.VMEM((NT, 1, 128), F32),
        pltpu.VMEM((NT, S, 128), BF16),
        pltpu.VMEM((3 * NT, D, 128), BF16),
        pltpu.VMEM((NT, D, 128), BF16),
        pltpu.VMEM((16, 256, 128), BF16),
        pltpu.VMEM((16, 128, 256), BF16),
        pltpu.VMEM((S, 128), BF16),
        pltpu.VMEM((16, 128, 256), BF16),
        pltpu.VMEM((16, 256, 256), F32),
        pltpu.VMEM((8, 128), F32),
        pltpu.VMEM((16, 256, 128), BF16),
        pltpu.VMEM((NT, S, 128), BF16),
        pltpu.VMEM((NT, 128, 128), F32),
        pltpu.VMEM((NT, 8, 128), F32),
        pltpu.VMEM((NT, D, 128), BF16),
        pltpu.VMEM((NT, 128, 128), BF16),
        pltpu.VMEM((NT, CH, 128), BF16),
        pltpu.VMEM((NT, S, 128), BF16),
        pltpu.SemaphoreType.DMA((44,)),
        pltpu.SemaphoreType.DMA((NT, 4)),
        pltpu.SemaphoreType.DMA((1 + NC, NT)),
    ]
    out = pl.pallas_call(
        _kernel,
        out_shape=jax.ShapeDtypeStruct((S, 2 * D), BF16),
        in_specs=[any_spec] * 11,
        out_specs=any_spec,
        scratch_shapes=scratch,
        compiler_params=pltpu.CompilerParams(vmem_limit_bytes=100 * 2**20),
    )(A_q[0], A_k[0], A_v[0], sk, A_ssm_k, sd, B_x[0], B_wqkv, B_wo,
      jnp.asarray(W1), jnp.asarray(WI))
    return out[None]
```

```python
import functools
import jax
import jax.numpy as jnp
import numpy as np
import ml_dtypes
from jax import lax
import jax.experimental.pallas as pl
import jax.experimental.pallas.tpu as pltpu

S, D = 2048, 1024
NT = D // 128
CH = 512
NC = S // CH
F32, BF16, U32, I32 = jnp.float32, jnp.bfloat16, jnp.uint32, jnp.int32


def _consts():
    k1 = np.arange(128)
    n1 = np.arange(128)
    W1 = np.zeros((16, 256, 128), np.float64)
    WI = np.zeros((16, 128, 256), np.float64)
    row_re = 16 * (k1 // 8) + (k1 % 8)
    row_im = row_re + 8
    for n2 in range(16):
        ang = 2 * np.pi * (k1[:, None] + 0.25) * (16 * n1[None, :] + n2) / 2048.0
        W1[n2, row_re] = np.cos(ang)
        W1[n2, row_im] = -np.sin(ang)
        WI[n2][:, row_re] = np.cos(ang).T / 2048.0
        WI[n2][:, row_im] = -np.sin(ang).T / 2048.0
    return W1.astype(ml_dtypes.bfloat16), WI.astype(ml_dtypes.bfloat16)


def _r4(x0, x1, x2, x3, inv):
    s02 = (x0[0] + x2[0], x0[1] + x2[1])
    d02 = (x0[0] - x2[0], x0[1] - x2[1])
    s13 = (x1[0] + x3[0], x1[1] + x3[1])
    d13 = (x1[0] - x3[0], x1[1] - x3[1])
    y0 = (s02[0] + s13[0], s02[1] + s13[1])
    y2 = (s02[0] - s13[0], s02[1] - s13[1])
    ya = (d02[0] + d13[1], d02[1] - d13[0])
    yb = (d02[0] - d13[1], d02[1] + d13[0])
    return (y0, yb, y2, ya) if inv else (y0, ya, y2, yb)


def _tw(x, e, inv):
    e = e % 16
    if inv:
        e = (16 - e) % 16
    r, i = x
    if e == 0:
        return x
    if e == 4:
        return (i, -r)
    if e == 12:
        return (-i, r)
    c = float(np.cos(2 * np.pi * e / 16))
    s = float(np.sin(2 * np.pi * e / 16))
    if e % 4 == 2:
        if np.sign(c) == np.sign(s):
            return ((r + i) * c, (i - r) * c)
        return ((r - i) * c, (i + r) * c)
    return (r * c + i * s, i * c - r * s)


def _fft16(x, inv, nxt=None, tied=None):
    def tz(x0, x1):
        if nxt is None:
            return x0, x1
        t = nxt()
        return (tied(x0[0], t), x0[1]), (tied(x1[0], t), x1[1])
    T = [None] * 4
    for b in range(4):
        y = _r4(*tz(x[b], x[4 + b]), x[8 + b], x[12 + b], inv)
        T[b] = [_tw(y[ka], b * ka, inv) for ka in range(4)]
    out = [None] * 16
    for ka in range(4):
        y = _r4(*tz(T[0][ka], T[1][ka]), T[2][ka], T[3][ka], inv)
        for kb in range(4):
            out[ka + 4 * kb] = y[kb]
    return out


def _lo(u):
    return pltpu.unpack_elementwise(u, index=0, packed_dtype=BF16, unpacked_dtype=F32)


def _hi(u):
    return pltpu.unpack_elementwise(u, index=1, packed_dtype=BF16, unpacked_dtype=F32)


def _phi(t):
    return jnp.where(t > 0, t + 1.0, jnp.exp(t)) + 1e-6


def _kernel(q_h, k_h, v_h, sk_h, h_h, sd_h, x_h, w_h, wo_h, w1_h, wi_h, zr,
            o_h,
            qb, kb, vb, hb, skb, sdb, xb, wb, wob, w1b, wib,
            ht, kvb, xa, ha, hs, pb, oa, kvs, zs, kvw, zb, pqb, ob,
            sem_in, sem_a, sem_o, sem_x):
    def cp(src, dst, sem):
        return pltpu.make_async_copy(src, dst, sem)

    def a_copies(t):
        cs = pl.ds(pl.multiple_of(t * 128, 128), 128)
        return [
            cp(k_h.at[:, cs], kb.at[t, pl.ds(16, S)], sem_a.at[t, 0]),
            cp(v_h.at[:, cs], vb.at[t], sem_a.at[t, 1]),
            cp(h_h.at[cs, :], hb.at[t], sem_a.at[t, 2]),
            cp(q_h.at[:, cs], qb.at[t], sem_a.at[t, 3]),
        ]
    c_small = [cp(sk_h, skb, sem_in.at[0]), cp(sd_h, sdb, sem_in.at[1]),
               cp(w1_h, w1b, sem_in.at[2]), cp(wi_h, wib, sem_in.at[3])]
    def c_x(c):
        rows = pl.ds(pl.multiple_of(c * CH, CH), CH)
        return [cp(x_h.at[rows, pl.ds(t * 128, 128)], xb.at[t, rows], sem_x.at[c, t]) for t in range(NT)]
    c_w = [cp(w_h.at[:, pl.ds(n * 128, 128)], wb.at[n], sem_in.at[12 + n]) for n in range(3 * NT)]
    c_wo = [cp(wo_h.at[:, pl.ds(n * 128, 128)], wob.at[n], sem_in.at[36 + n]) for n in range(NT)]
    for c in c_small[:3] + a_copies(0)[:3] + c_x(0) + c_w[NT:]:
        c.start()
    for t in range(NT):
        kb[t, 0:16, :] = jnp.zeros((16, 128), BF16)
    for c in c_small[:3]:
        c.wait()

    kbu = kb.bitcast(U32)
    vbu = vb.bitcast(U32)
    qbu = qb.bitcast(U32)
    htu = ht.bitcast(U32)
    oau = oa.bitcast(U32)


    zero = zr[...]

    class Tie:
        def __init__(self, parts, lo, hi, n):
            self.parts, self.n, self.c = parts, n, 0
            tot = len(parts) * (CH // 8)
            self.lo, self.hi = int(lo * tot), int(hi * tot)
        def next(self):
            p = self.lo + (self.c * (self.hi - self.lo)) // self.n
            self.c += 1
            assert self.c <= self.n
            part = self.parts[p // (CH // 8)]
            r = (p % (CH // 8)) * 8
            return pltpu.bitcast(part[r:r + 8], I32) & zero
    def tied(x, t):
        if t is None:
            return x
        if x.shape[0] != 8:
            t = jnp.concatenate([t] * (x.shape[0] // 8), axis=0)
        return pltpu.bitcast(pltpu.bitcast(x, I32) | t, x.dtype)

    def prep_conv(t, tie):
        wf = skb[t].astype(F32)
        w = [wf[j:j + 1, :] for j in range(4)]
        for j in range(8):
            base = 8 * 16 * j + 8
            kk = {}
            for m in range(-2, 8):
                u = kbu[t, pl.ds(base + m, 16, stride=8), :]
                if m % 3 == 1:
                    u = tied(u, tie.next() if tie else None)
                kk[2 * m] = _lo(u)
                kk[2 * m + 1] = _hi(u)
            for m in range(8):
                u = vbu[t, pl.ds(base - 8 + m, 16, stride=8), :]
                for n2, vv in ((2 * m, _lo(u)), (2 * m + 1, _hi(u))):
                    ks = kk[n2] * w[0] + kk[n2 - 1] * w[1] + kk[n2 - 2] * w[2] + kk[n2 - 3] * w[3]
                    kvb[t, n2, 16 * j:16 * j + 16, :] = (ks * vv).astype(BF16)

    def prep_h(t):
        ht[...] = hb[t].T
        for m in range(8):
            u = htu[pl.ds(m, 128, stride=8), :]
            hs[2 * m] = _lo(u).astype(BF16)
            hs[2 * m + 1] = _hi(u).astype(BF16)

    def prep_f1(t, s):
        for n2 in range(16):
            xa[s, n2] = jnp.dot(w1b[n2], kvb[t, n2], preferred_element_type=F32)
            ha[s, n2] = jnp.dot(w1b[n2], hs[n2], preferred_element_type=F32)

    def fft(s, tie):
        nxt = (lambda: tie.next()) if tie else None
        tf = (lambda x0, x1: None) if tie is None else None
        for g in range(16):
            r0, r1, r2 = 16 * g, 16 * g + 8, 16 * g + 16
            H = _fft16([(ha[s, n, r0:r1], ha[s, n, r1:r2]) for n in range(16)], False, nxt, tied)
            for n in range(16):
                ha[s, n, r0:r1] = H[n][0]
                ha[s, n, r1:r2] = H[n][1]
            X = _fft16([(xa[s, n, r0:r1], xa[s, n, r1:r2]) for n in range(16)], False, nxt, tied)
            P = []
            for n in range(16):
                hr, hi = ha[s, n, r0:r1], ha[s, n, r1:r2]
                P.append((X[n][0] * hr - X[n][1] * hi, X[n][0] * hi + X[n][1] * hr))
            Y = _fft16(P, True, nxt, tied)
            for n in range(16):
                pb[s, n, r0:r2, :] = jnp.concatenate(Y[n], axis=0).astype(BF16)

    def fin(t, s):
        dd = sdb[:, pl.ds(pl.multiple_of(t * 128, 128), 128)].astype(F32)
        for m in range(8):
            u = qbu[t, pl.ds(m, 128, stride=8), :]
            res = []
            for n2, qq in ((2 * m, _lo(u)), (2 * m + 1, _hi(u))):
                y = jnp.dot(wib[n2], pb[s, n2], preferred_element_type=F32)
                y = y + kvb[t, n2].astype(F32) * dd
                res.append(y * qq)
            oau[t, pl.ds(m, 128, stride=8), :] = pltpu.pack_elementwise(res, packed_dtype=BF16)

    def a_out(t):
        cs = pl.ds(pl.multiple_of(t * 128, 128), 128)
        return cp(oa.at[t], o_h.at[:, cs], sem_o.at[0, t])

    def a_step(i, parts):
        tn = jnp.minimum(i + 1, NT - 1)
        tp = jnp.maximum(i - 1, 0)
        fft(i % 2, Tie(parts, 0.03, 0.93, 16 * 24))
        prep_conv(tn, Tie(parts, 0.1, 0.9, 32))
        prep_h(tn)
        prep_f1(tn, (i + 1) % 2)

    def a_pre(i):
        @pl.when(i + 1 < NT)
        def _():
            for c in a_copies(i + 1):
                c.wait()

        @pl.when(i + 2 < NT)
        def _():
            for c in a_copies(i + 2):
                c.start()

    def a_post(i):
        @pl.when(i > 0)
        def _():
            a_out(i - 1).start()

    pb[1] = jnp.zeros(pb.shape[1:], BF16)
    kvs[...] = jnp.zeros(kvs.shape, F32)
    zs[...] = jnp.zeros(zs.shape, F32)
    for c in a_copies(0)[:3]:
        c.wait()
    for c in c_small[3:] + a_copies(0)[3:] + a_copies(1):
        c.start()
    prep_conv(0, None)
    prep_h(0)
    prep_f1(0, 0)
    for c in c_w[NT:] + c_small[3:] + a_copies(0)[3:]:
        c.wait()
    for c in c_w[:NT] + c_wo:
        c.start()

    def proj(rows, n, parts):
        acc = None
        for k in range(NT):
            p = jnp.dot(xb[k, rows, :], wb[n, k * 128:(k + 1) * 128, :], preferred_element_type=F32)
            parts.append(p)
            acc = p if acc is None else acc + p
        return acc

    def b1(c, carry):
        for cc in c_x(c):
            cc.wait()

        @pl.when(c + 1 < NC)
        def _():
            for cc in c_x(c + 1):
                cc.start()
        a_pre(c)
        fin(jnp.maximum(c - 1, 0), (c + 1) % 2)
        rows = pl.ds(pl.multiple_of(c * CH, CH), CH)
        parts, pend = [], []

        def kvacc(n, a, b):
            kvs[n] += lax.dot_general(a, b, (((0,), (0,)), ((), ())), preferred_element_type=F32)
        for n in range(NT):
            pk = _phi(proj(rows, NT + n, parts))
            zs[n] += jnp.sum(pk.reshape(CH // 8, 8, 128), axis=0)
            pkb = pk.astype(BF16)
            if pend:
                kvacc(*pend.pop())
            pend.append((n, pkb, proj(rows, 2 * NT + n, parts).astype(BF16)))
        kvacc(*pend.pop())
        a_step(c, parts)
        a_post(c)
        return carry

    lax.fori_loop(0, NC, b1, 0)

    for c in c_wo + c_w[:NT]:
        c.wait()
    ri = lax.broadcasted_iota(I32, (128, 128), 0)
    ci = lax.broadcasted_iota(I32, (128, 128), 1)
    mask = (ri // 32) == (ci // 32)
    for g in range(NT):
        kvm = jnp.where(mask, kvs[g], 0.0).astype(BF16)
        for n in range(NT):
            kvw[n, g * 128:(g + 1) * 128, :] = jnp.dot(
                kvm, wob[n, g * 128:(g + 1) * 128, :], preferred_element_type=F32).astype(BF16)
        z = jnp.sum(zs[g], axis=0, keepdims=True)
        zt = jnp.broadcast_to(z, (128, 128)).T
        zb[g] = jnp.where(mask, zt, 0.0).astype(BF16)

    def b3(c, carry):
        a_pre(c + NC)
        fin(c + NC - 1, (c + 1) % 2)
        rows = pl.ds(pl.multiple_of(c * CH, CH), CH)
        parts = []
        prev = None
        for g in range(NT + 1):
            if g < NT:
                cur = _phi(proj(rows, g, parts)).astype(BF16)
            if prev is not None:
                den = jnp.dot(prev, zb[g - 1], preferred_element_type=F32) + 1e-6
                pqb[g - 1] = (prev.astype(F32) / den).astype(BF16)
            prev = cur
        for n in range(NT):
            acc = None
            for g in range(NT):
                p = jnp.dot(pqb[g], kvw[n, g * 128:(g + 1) * 128, :], preferred_element_type=F32)
                parts.append(p)
                acc = p if acc is None else acc + p
            ob[n, rows, :] = acc.astype(BF16)
        a_step(c + NC, parts)
        for n in range(NT):
            cp(ob.at[n, rows], o_h.at[rows, pl.ds(D + n * 128, 128)], sem_o.at[1 + c, n]).start()
        a_out(c + NC - 1).start()
        return carry

    lax.fori_loop(0, NC, b3, 0)
    fin(NT - 1, (NT - 1) % 2)
    a_out(NT - 1).start()

    for t in range(NT):
        a_out(t).wait()
        for c in range(NC):
            rows = pl.ds(c * CH, CH)
            cp(ob.at[t, rows], o_h.at[rows, pl.ds(D + t * 128, 128)], sem_o.at[1 + c, t]).wait()


@jax.jit
def pallas_concat_heads__ssm_conv_h3__linear_attn_block__prompt_kernel(
        A_q, A_k, A_v, A_shift_k, A_ssm_k, A_ssm_D, B_x, B_wqkv, B_wo):
    W1, WI = _consts()
    sk = A_shift_k.T.reshape(4, NT, 128).transpose(1, 0, 2)
    sd = A_ssm_D.reshape(1, D)
    any_spec = pl.BlockSpec(memory_space=pl.ANY)
    scratch = [
        pltpu.VMEM((NT, S, 128), BF16),
        pltpu.VMEM((NT, S + 16, 128), BF16),
        pltpu.VMEM((NT, S, 128), BF16),
        pltpu.VMEM((NT, 128, S), BF16),
        pltpu.VMEM((NT, 4, 128), BF16),
        pltpu.VMEM((1, D), BF16),
        pltpu.VMEM((NT, S, 128), BF16),
        pltpu.VMEM((3 * NT, D, 128), BF16),
        pltpu.VMEM((NT, D, 128), BF16),
        pltpu.VMEM((16, 256, 128), BF16),
        pltpu.VMEM((16, 128, 256), BF16),
        pltpu.VMEM((S, 128), BF16),
        pltpu.VMEM((NT, 16, 128, 128), BF16),
        pltpu.VMEM((2, 16, 256, 128), F32),
        pltpu.VMEM((2, 16, 256, 128), F32),
        pltpu.VMEM((16, 128, 128), BF16),
        pltpu.VMEM((2, 16, 256, 128), BF16),
        pltpu.VMEM((NT, S, 128), BF16),
        pltpu.VMEM((NT, 128, 128), F32),
        pltpu.VMEM((NT, 8, 128), F32),
        pltpu.VMEM((NT, D, 128), BF16),
        pltpu.VMEM((NT, 128, 128), BF16),
        pltpu.VMEM((NT, CH, 128), BF16),
        pltpu.VMEM((NT, S, 128), BF16),
        pltpu.SemaphoreType.DMA((44,)),
        pltpu.SemaphoreType.DMA((NT, 4)),
        pltpu.SemaphoreType.DMA((1 + NC, NT)),
        pltpu.SemaphoreType.DMA((NC, NT)),
    ]
    out = pl.pallas_call(
        _kernel,
        out_shape=jax.ShapeDtypeStruct((S, 2 * D), BF16),
        in_specs=[any_spec] * 11 + [pl.BlockSpec(memory_space=pltpu.VMEM)],
        out_specs=any_spec,
        scratch_shapes=scratch,
        compiler_params=pltpu.CompilerParams(vmem_limit_bytes=100 * 2**20),
    )(A_q[0], A_k[0], A_v[0], sk, A_ssm_k, sd, B_x[0], B_wqkv, B_wo,
      jnp.asarray(W1), jnp.asarray(WI), jnp.asarray(np.zeros((8, 128), np.int32)))
    return out[None]
```
